```python
import jax
import jax.numpy as jnp

def _softmax(x, axis=-1):
    return jax.nn.softmax(x, axis=axis)

def _gelu(x):
    return jax.nn.gelu(x, approximate=True)

def _silu(x):
    return jax.nn.silu(x)

def _sigmoid(x):
    return jax.nn.sigmoid(x)

def _layernorm(x, axis=-1, eps=1e-05):
    m = jnp.mean(x, axis=axis, keepdims=True)
    v = jnp.var(x, axis=axis, keepdims=True)
    return (x - m) / jnp.sqrt(v + eps)

def _scatter_add(tgt, idx, src, axis=0):
    return tgt.at[idx].add(src)

def _segment_sum(src, seg, n):
    return jax.ops.segment_sum(src, seg, n)

class _Rng:

    def __init__(self, key):
        self._k = key

    def _next(self):
        self._k, sub = jax.random.split(self._k)
        return sub

    def normal(self, shape):
        return jax.random.normal(self._next(), shape, dtype=jnp.bfloat16)

    def randint(self, lo, hi, shape):
        return jax.random.randint(self._next(), shape, lo, hi, dtype=jnp.int32)

    def uniform(self, shape, lo=0.0, hi=1.0):
        return jax.random.uniform(self._next(), shape, jnp.bfloat16, lo, hi)

    def permutation(self, n):
        return jax.random.permutation(self._next(), n)
kernel_name = 'adaLN_cond__mha_block_cached__moe_arch_mod__prompt'

def setup_inputs():
    _rng = _Rng(jax.random.key(int.from_bytes(__import__("os").urandom(4), "little")))
    _w = lambda a: (lambda t: t.astype(jnp.bfloat16) if jnp.issubdtype(t.dtype, jnp.floating) else t)(jnp.asarray(a))

    def _A_setup():
        B, Sq, D = (1, 2048, 1024)
        H, Sk, Dh = (32, 2048, 128)
        return {'x': _w((lambda *s: _rng.normal(s) * 0.05)(B, Sq, D)), 'k_cache': _w((lambda *s: _rng.normal(s) * 0.05)(B, H, Sk, Dh)), 'v_cache': _w((lambda *s: _rng.normal(s) * 0.05)(B, H, Sk, Dh)), 'wq': _w((lambda *s: _rng.normal(s) * 0.05)(D, H * Dh) * D ** (-0.5)), 'wo': _w((lambda *s: _rng.normal(s) * 0.05)(H * Dh, D) * (H * Dh) ** (-0.5))}
    _A_in = _A_setup()

    def _B_setup():
        B, S, D, F, C = (1, 2048, 1024, 3584, 2)
        return {'x': _w((lambda *s: _rng.normal(s) * 0.05)(B, S, D)), 'w_r': _w((lambda *s: _rng.normal(s) * 0.05)(D)), 'w_gate': _w((lambda *s: _rng.normal(s) * 0.05)(D, F)), 'w_up': _w((lambda *s: _rng.normal(s) * 0.05)(D, F)), 'w_down': _w((lambda *s: _rng.normal(s) * 0.05)(F, D))}
    _B_in = _B_setup()
    return {'A_x': _A_in['x'], 'A_k_cache': _A_in['k_cache'], 'A_v_cache': _A_in['v_cache'], 'A_wq': _A_in['wq'], 'A_wo': _A_in['wo'], 'B_x': _B_in['x'], 'B_w_r': _B_in['w_r'], 'B_w_gate': _B_in['w_gate'], 'B_w_up': _B_in['w_up'], 'B_w_down': _B_in['w_down'], 'c': _w((lambda *s: _rng.normal(s) * 0.05)(1, 1024)), 'w_mod': _w((lambda *s: _rng.normal(s) * 0.05)(1024, 6 * 1024) * 1024 ** (-0.5))}

def reference(A_x, A_k_cache, A_v_cache, A_wq, A_wo, B_x, B_w_r, B_w_gate, B_w_up, B_w_down, c, w_mod):

    def _A_ref(x, k_cache, v_cache, wq, wo):
        B, Sq, D = x.shape
        H, Dh = (32, 128)
        q = (lambda x, *d: x.transpose(*d))((x @ wq).reshape(B, Sq, H, Dh), 0, 2, 1, 3)
        scores = jnp.einsum('bhqd,bhkd->bhqk', q, k_cache) * Dh ** (-0.5)
        p = _softmax(scores, axis=-1)
        o = jnp.einsum('bhqk,bhkd->bhqd', p, v_cache)
        return (lambda x, *d: x.transpose(*d))(o, 0, 2, 1, 3).reshape(B, Sq, H * Dh) @ wo

    def _B_ref(x, w_r, w_gate, w_up, w_down):
        B, S, D = x.shape
        C = 2
        r = x @ w_r
        idx = jnp.argsort(-r, axis=-1)[:, :C]
        idx_e = jnp.repeat(idx.reshape(B, C, 1), D, axis=2)
        x_sel = jnp.take_along_axis(x, idx_e, axis=1)
        g = _silu(x_sel @ w_gate)
        u = x_sel @ w_up
        y = g * u @ w_down
        r_sel = _sigmoid(jnp.take_along_axis(r, idx, axis=1))
        y = y * r_sel.reshape(B, C, 1)
        b_off = (jnp.arange(B) * S).reshape(B, 1)
        flat_idx = (idx + b_off).reshape(B * C)
        zero = (x * 0.0).reshape(B * S, D)
        upd = _scatter_add(zero, flat_idx, y.reshape(B * C, D), axis=0)
        return x + upd.reshape(B, S, D)
    x = A_x
    mod = (_silu(c) @ w_mod).reshape(c.shape[0], 6, 1, -1)
    sa, ca, ga, sb, cb, gb = (mod[:, 0].copy(), mod[:, 1].copy(), mod[:, 2].copy(), mod[:, 3].copy(), mod[:, 4].copy(), mod[:, 5].copy())
    h = _layernorm(x, axis=-1) * (1 + ca) + sa
    x = x + ga * _A_ref(h, A_k_cache, A_v_cache, A_wq, A_wo)
    h = _layernorm(x, axis=-1) * (1 + cb) + sb
    x = x + gb * _B_ref(h, B_w_r, B_w_gate, B_w_up, B_w_down)
    return x
```

```python
import functools
import math

import jax
import jax.numpy as jnp
from jax import lax
import jax.experimental.pallas as pl
import jax.experimental.pallas.tpu as pltpu

S = 2048
D = 1024
H = 32
DH = 128
F = 3584
BQ = 256
NQ = S // BQ
LNB = 256
EPS = 1e-5
Q_SCALE = (DH ** -0.5) * math.log2(math.e)

BF16 = jnp.bfloat16
F32 = jnp.float32
NT = (((1,), (1,)), ((), ()))


def _dot(a, b):
    return jnp.dot(a, b, preferred_element_type=F32)


def _layernorm(x):
    m = jnp.mean(x, axis=1, keepdims=True)
    xc = x - m
    v = jnp.mean(xc * xc, axis=1, keepdims=True)
    return xc * lax.rsqrt(v + EPS)


def _kernel(x_hbm, k_hbm, v_hbm, wq_hbm, wo_hbm, wr_hbm, wg_hbm, wu_hbm, wd_hbm, c_hbm, wm_hbm,
            out_hbm,
            x_v, h_v, acc_v, k_v, v_v, wq_v, wo_v, wm_v, wg_v, wu_v, wd_v, c_v, wr_v, mod_v,
            r_v, o_v, p_v,
            head_sem, x_sem, wm_sem, ffn_sem, misc_sem, out_sem):

    def head_copies(h, slot):
        col = pl.ds(pl.multiple_of(h * DH, DH), DH)
        return (
            pltpu.make_async_copy(wq_hbm.at[:, col], wq_v.at[slot], head_sem.at[0, slot]),
            pltpu.make_async_copy(k_hbm.at[0, h], k_v.at[slot], head_sem.at[1, slot]),
            pltpu.make_async_copy(v_hbm.at[0, h], v_v.at[slot], head_sem.at[2, slot]),
            pltpu.make_async_copy(wo_hbm.at[col, :], wo_v.at[slot], head_sem.at[3, slot]),
        )

    def x_copy(i):
        rows = pl.ds(i * LNB, LNB)
        return pltpu.make_async_copy(x_hbm.at[0, rows, :], x_v.at[rows, :], x_sem.at[i])

    def wm_copy(j):
        cols = pl.ds(j * D, D)
        return pltpu.make_async_copy(wm_hbm.at[:, cols], wm_v.at[:, cols], wm_sem.at[j])

    def out_copy(i):
        rows = pl.ds(i * LNB, LNB)
        return pltpu.make_async_copy(o_v.at[rows, :], out_hbm.at[0, rows, :], out_sem.at[i])

    c_copy = pltpu.make_async_copy(c_hbm, c_v, misc_sem.at[0])
    wr_copy = pltpu.make_async_copy(wr_hbm, wr_v, misc_sem.at[1])
    ffn_copies = (
        pltpu.make_async_copy(wg_hbm, wg_v, ffn_sem.at[0]),
        pltpu.make_async_copy(wu_hbm, wu_v, ffn_sem.at[1]),
        pltpu.make_async_copy(wd_hbm, wd_v, ffn_sem.at[2]),
    )

    c_copy.start()
    wm_copy(1).start()
    wm_copy(0).start()
    for i in range(S // LNB):
        x_copy(i).start()
    for cp in head_copies(0, 0):
        cp.start()
    wr_copy.start()

    c_copy.wait()
    c32 = c_v[...].astype(F32)
    sc = jnp.broadcast_to((c32 * jax.nn.sigmoid(c32)).astype(BF16), (16, D))

    def mod_chunk(j):
        wm_copy(j).wait()
        mod_v[:, j * D:(j + 1) * D] = _dot(sc, wm_v[:, j * D:(j + 1) * D])[0:8]

    mod_chunk(1)
    mod_chunk(0)

    def mod(j):
        return mod_v[0:1, j * D:(j + 1) * D]

    for i in range(S // LNB):
        x_copy(i).wait()
        rows = pl.ds(i * LNB, LNB)
        xn = _layernorm(x_v[rows, :].astype(F32))
        h_v[rows, :] = (xn * (1.0 + mod(1)) + mod(0)).astype(BF16)
        acc_v[rows, :] = jnp.zeros((LNB, D), F32)

    def head_body(h, carry):
        slot = h % 2

        @pl.when(h + 1 < H)
        def _():
            for cp in head_copies(h + 1, 1 - slot):
                cp.start()

        @pl.when(h == 1)
        def _():
            ffn_copies[0].start()

        @pl.when(h == 3)
        def _():
            ffn_copies[1].start()

        @pl.when(h == 5)
        def _():
            ffn_copies[2].start()

        @pl.when(h == 7)
        def _():
            for j in range(2, 6):
                wm_copy(j).start()

        @pl.when(h == 10)
        def _():
            c32_ = c_v[...].astype(F32)
            sc_ = jnp.broadcast_to((c32_ * jax.nn.sigmoid(c32_)).astype(BF16), (16, D))
            for j in range(2, 6):
                wm_copy(j).wait()
                mod_v[:, j * D:(j + 1) * D] = _dot(sc_, wm_v[:, j * D:(j + 1) * D])[0:8]

        for cp in head_copies(h, slot):
            cp.wait()

        for i in range(NQ):
            rows = pl.ds(i * BQ, BQ)
            q = (_dot(h_v[rows, :], wq_v[slot]) * Q_SCALE).astype(BF16)
            s = lax.dot_general(q, k_v[slot], NT, preferred_element_type=F32)
            m = jnp.max(s, axis=1, keepdims=True)
            p = jnp.exp2(s - m)
            l = jnp.sum(p, axis=1, keepdims=True)
            o = _dot(p.astype(BF16), v_v[slot])
            o = (o / l).astype(BF16)
            acc_v[rows, :] += _dot(o, wo_v[slot])
        return carry

    lax.fori_loop(0, H, head_body, 0)

    wr_copy.wait()
    wr = jnp.concatenate([wr_v[j:j + 1, :] for j in range(D // 128)], axis=1).astype(F32)
    for i in range(S // LNB):
        rows = pl.ds(i * LNB, LNB)
        x1 = x_v[rows, :].astype(F32) + mod(2) * acc_v[rows, :]
        h2 = (_layernorm(x1) * (1.0 + mod(4)) + mod(3)).astype(BF16)
        h_v[rows, :] = h2
        h2 = h2.astype(F32)
        r = jnp.sum(h2 * wr, axis=1, keepdims=True)
        r_v[rows, :] = jnp.broadcast_to(r, (LNB, 128))
        base = x1 + mod(5) * (h2 + h2 * 0.0)
        acc_v[rows, :] = base
        o_v[rows, :] = base.astype(BF16)
        out_copy(i).start()

    r = r_v[...]
    row_id = lax.broadcasted_iota(jnp.int32, (S, 128), 0)
    m1 = jnp.max(r, axis=0, keepdims=True)
    i1 = jnp.min(jnp.where(r == m1, row_id, S), axis=0, keepdims=True)
    r2 = jnp.where(row_id == i1, -jnp.inf, r)
    m2 = jnp.max(r2, axis=0, keepdims=True)
    i2 = jnp.min(jnp.where((r2 == m2) & (row_id != i1), row_id, S), axis=0, keepdims=True)
    idx1 = jnp.minimum(i1[0, 0], S - 1)
    idx2 = jnp.minimum(i2[0, 0], S - 1)

    def slab(idx):
        return pl.ds(pl.multiple_of((idx // 16) * 16, 16), 16)

    sub = lax.broadcasted_iota(jnp.int32, (16, D), 0)

    def pick_row(idx):
        rows = h_v[slab(idx), :].astype(F32)
        return jnp.sum(jnp.where(sub == idx % 16, rows, 0.0), axis=0, keepdims=True)

    xs = jnp.where(sub == 0, pick_row(idx1), jnp.where(sub == 1, pick_row(idx2), 0.0)).astype(BF16)

    ffn_copies[0].wait()
    g = _dot(xs, wg_v[...])
    ffn_copies[1].wait()
    u = _dot(xs, wu_v[...])
    a = (g * jax.nn.sigmoid(g) * u).astype(BF16)
    ffn_copies[2].wait()
    y = _dot(a, wd_v[...])
    gb = mod(5)
    d1 = gb * (y[0:1] * jax.nn.sigmoid(m1[:, 0:1]))
    d2 = gb * (y[1:2] * jax.nn.sigmoid(m2[:, 0:1]))

    for i in range(S // LNB):
        out_copy(i).wait()

    for idx, d in ((idx1, d1), (idx2, d2)):
        rows = slab(idx)
        acc_v[rows, :] = acc_v[rows, :] + jnp.where(sub == idx % 16, d, 0.0)
    for n, idx in enumerate((idx1, idx2)):
        rows = slab(idx)
        p_v[...] = acc_v[rows, :].astype(BF16)
        cp = pltpu.make_async_copy(p_v, out_hbm.at[0, rows, :], misc_sem.at[2])
        cp.start()
        cp.wait()


@jax.jit
def pallas_adaLN_cond__mha_block_cached__moe_arch_mod__prompt_kernel(
    A_x: jax.Array,
    A_k_cache: jax.Array,
    A_v_cache: jax.Array,
    A_wq: jax.Array,
    A_wo: jax.Array,
    B_x: jax.Array,
    B_w_r: jax.Array,
    B_w_gate: jax.Array,
    B_w_up: jax.Array,
    B_w_down: jax.Array,
    c: jax.Array,
    w_mod: jax.Array,
):
    del B_x
    any_spec = pl.BlockSpec(memory_space=pl.ANY)
    scratch = [
        pltpu.VMEM((S, D), BF16),
        pltpu.VMEM((S, D), BF16),
        pltpu.VMEM((S, D), F32),
        pltpu.VMEM((2, S, DH), BF16),
        pltpu.VMEM((2, S, DH), BF16),
        pltpu.VMEM((2, D, DH), BF16),
        pltpu.VMEM((2, DH, D), BF16),
        pltpu.VMEM((D, 6 * D), BF16),
        pltpu.VMEM((D, F), BF16),
        pltpu.VMEM((D, F), BF16),
        pltpu.VMEM((F, D), BF16),
        pltpu.VMEM((1, D), BF16),
        pltpu.VMEM((D // 128, 128), BF16),
        pltpu.VMEM((8, 6 * D), F32),
        pltpu.VMEM((S, 128), F32),
        pltpu.VMEM((S, D), BF16),
        pltpu.VMEM((16, D), BF16),
        pltpu.SemaphoreType.DMA((4, 2)),
        pltpu.SemaphoreType.DMA((S // LNB,)),
        pltpu.SemaphoreType.DMA((6,)),
        pltpu.SemaphoreType.DMA((3,)),
        pltpu.SemaphoreType.DMA((3,)),
        pltpu.SemaphoreType.DMA((S // LNB,)),
    ]
    return pl.pallas_call(
        _kernel,
        out_shape=jax.ShapeDtypeStruct((1, S, D), BF16),
        in_specs=[any_spec] * 11,
        out_specs=any_spec,
        scratch_shapes=scratch,
        compiler_params=pltpu.CompilerParams(vmem_limit_bytes=110 * 1024 * 1024),
    )(A_x, A_k_cache, A_v_cache, A_wq, A_wo, B_w_r.reshape(D // 128, 128), B_w_gate, B_w_up, B_w_down,
      c, w_mod)
```

```python
import functools
import math

import jax
import jax.numpy as jnp
from jax import lax
import jax.experimental.pallas as pl
import jax.experimental.pallas.tpu as pltpu

S = 2048
D = 1024
H = 32
DH = 128
F = 3584
BQ = 256
BK = 512
RB1 = 256
NP1 = 7
WC = 512
NKC = 2
RB3 = 128
NP3 = 16
UNROLL = 2
EPS = 1e-5
Q_SCALE = (DH ** -0.5) * math.log2(math.e)
L_MIN = 2.0 ** -30
L_MAX = 2.0 ** 64
VMEM_MB = 122
NOBC = True
FAST = True
PAD = 128
PADM = 128

BF16 = jnp.bfloat16
F32 = jnp.float32
I32 = jnp.int32
NT = (((1,), (1,)), ((), ()))


def _pieces(rows, n):
    unit = 16 if rows // 16 >= n else 8
    units = rows // unit
    return [unit * (units // n + (1 if c < units % n else 0)) for c in range(n)]


def _dot(a, b):
    return jnp.dot(a, b, preferred_element_type=F32)


def _qk(q, k):
    return lax.dot_general(q, k, NT, preferred_element_type=F32)


def _attn_head_fast(q_ref, k_ref, v_ref, o_ref):
    bad = jnp.zeros((8, DH), F32)
    for i in range(S // BQ):
        rows = slice(i * BQ, (i + 1) * BQ)
        q = q_ref[rows, :]
        acc = l = None
        for a in range(0, S, BK):
            p = jnp.exp2(_qk(q, k_ref[a:a + BK, :]))
            for t in range(BK // DH):
                pt = p[:, t * DH:(t + 1) * DH]
                l = pt if l is None else l + pt
            pv = _dot(p.astype(BF16), v_ref[a:a + BK, :])
            acc = pv if acc is None else acc + pv
        l = jnp.sum(l, axis=1, keepdims=True)
        o = acc * jnp.where((l >= L_MIN) & (l <= L_MAX), 1.0 / l, jnp.nan)
        o_ref[rows, :] = o.astype(BF16)
        z = o * 0.0
        for t in range(BQ // 8):
            bad = bad + z[t * 8:(t + 1) * 8]
    return bad


def _attn_head_exact(q_ref, k_ref, v_ref, o_ref):
    def body(i, carry):
        rows = pl.ds(pl.multiple_of(i * BQ, BQ), BQ)
        s = _qk(q_ref[rows, :], k_ref[...])
        p = jnp.exp2(s - jnp.max(s, axis=1, keepdims=True))
        l = jnp.sum(p, axis=1, keepdims=True)
        o_ref[rows, :] = (_dot(p.astype(BF16), v_ref[...]) / l).astype(BF16)
        return carry
    lax.fori_loop(0, S // BQ, body, 0)


def _kernel(x_hbm, k_hbm, v_hbm, wq_hbm, wo_hbm, wr_hbm, wg_hbm, wu_hbm, wd_hbm, c_hbm, wm_hbm,
            out_hbm,
            x_v, ha_v, hb_v, q_v, o_v, k_v, v_v, wq_v, wo_v, wm_v, wg_v, wu_v, wd_v, c_v, wr_v, mod_v,
            att_a, att_b, y_v, zero_v,
            kv_sem, x_sem, wa_sem, wq_sem, w_sem, misc_sem, out_sem, fence_sem):
    NB1 = S // RB1
    NB3 = S // RB3
    NWC = H * DH // WC
    HPC = WC // DH
    NS = 2 * UNROLL
    KC = D // NKC

    def kv_copies(h, slot):
        return (
            pltpu.make_async_copy(k_hbm.at[0, h], k_v.at[slot], kv_sem.at[0, slot]),
            pltpu.make_async_copy(v_hbm.at[0, h], v_v.at[slot], kv_sem.at[1, slot]),
        )

    def x_copy(i):
        rows = pl.ds(pl.multiple_of(i * RB1, RB1), RB1)
        return pltpu.make_async_copy(x_hbm.at[0, rows, :], x_v.at[rows, :], x_sem.at[i])

    def wa_copy(j):
        rows = pl.ds(j * KC, KC)
        return pltpu.make_async_copy(wm_hbm.at[rows, 0:2 * D], wm_v.at[rows, 0:2 * D], wa_sem.at[j])

    def wq_copy(j):
        cols = pl.ds(pl.multiple_of(j * WC, WC), WC)
        return pltpu.make_async_copy(wq_hbm.at[:, cols], wq_v.at[j], wq_sem.at[j])

    def out_copy(i):
        rows = pl.ds(pl.multiple_of(i * RB3, RB3), RB3)
        return pltpu.make_async_copy(y_v.at[rows, 0:D], out_hbm.at[0, rows, :], out_sem.at[i])

    c_copy = pltpu.make_async_copy(c_hbm, c_v, misc_sem.at[0])
    wr2_copy = pltpu.make_async_copy(wm_hbm.at[:, 2 * D:6 * D], wm_v.at[:, 2 * D:6 * D], misc_sem.at[4])
    wr_copy = pltpu.make_async_copy(wr_hbm, wr_v, misc_sem.at[1])
    wo_copy = pltpu.make_async_copy(wo_hbm, wo_v, w_sem.at[0])
    wg_copy = pltpu.make_async_copy(wg_hbm, wg_v, w_sem.at[1])
    wu_copy = pltpu.make_async_copy(wu_hbm, wu_v, w_sem.at[2])
    wd_copy = pltpu.make_async_copy(wd_hbm, wd_v.at[:, 0:D], w_sem.at[3])

    def after(val, dep):
        if dep is None:
            return val
        dep = jnp.tile(dep, (val.shape[0] // 8, 1))
        return lax.bitcast_convert_type(lax.bitcast_convert_type(val, I32) | dep, F32)

    def mark(val):
        return lax.bitcast_convert_type(val[val.shape[0] - 8:], I32) & zero_v[:, 0:1]

    def layernorm(x, dep, n=None):
        m = after(jnp.mean(x, axis=1, keepdims=True), dep)
        xc = x - m
        v = jnp.mean(xc * xc, axis=1, keepdims=True)
        return xc * lax.rsqrt(v + EPS), v

    def mod(j):
        return mod_v[0:1, j * D:(j + 1) * D]

    def silu_c():
        c32 = c_v[...].astype(F32)
        return jnp.broadcast_to((c32 * jax.nn.sigmoid(c32)).astype(BF16), (16, D))

    def in_order(copies):
        for cp in copies:
            cp.start()
            pl.semaphore_signal(fence_sem, 1)
            pl.semaphore_wait(fence_sem, 1)

    in_order([c_copy, x_copy(0)] + [wa_copy(j) for j in range(NKC)] + [wq_copy(0)]
             + [x_copy(i) for i in range(1, NB1)])
    zero_v[...] = jnp.zeros((8, DH), I32)
    att_b[...] = jnp.zeros((RB3, D), F32)

    with jax.named_scope('c'):
        c_copy.wait()
        sc = silu_c()
    with jax.named_scope('x0'):
        x_copy(0).wait()
        xn0, _ = layernorm(x_v[0:RB1, :].astype(F32), None)
    with jax.named_scope('moda'):
        acc = None
        for j in range(NKC):
            wa_copy(j).wait()
            part = _dot(sc[:, j * KC:(j + 1) * KC], wm_v[j * KC:(j + 1) * KC, 0:2 * D])
            acc = part if acc is None else acc + part
        mod_v[:, 0:2 * D] = acc[0:8]
        ha_v[0] = (xn0 * (1.0 + acc[0:1, D:2 * D]) + acc[0:1, 0:D]).astype(BF16)

    def ln1(i, dst, j):
        dep = None
        off = 0
        for n in _pieces(RB1, NP1):
            rows = pl.ds(pl.multiple_of(i * RB1 + off, 8), n)
            xn, v = layernorm(x_v[rows, :].astype(F32), dep, n)
            dst[j, off:off + n, :] = (xn * (1.0 + mod(1)) + mod(0)).astype(BF16)
            dep = mark(v)
            off += n

    def qproj(h, rows, j, t0=0, t1=HPC):
        q = _dot(h, wq_v[j, :, t0 * DH:t1 * DH])
        for t in range(t0, t1):
            q_v[j * HPC + t, rows, :] = (q[:, (t - t0) * DH:(t - t0 + 1) * DH] * Q_SCALE).astype(BF16)

    def block(i):
        return pl.ds(pl.multiple_of(i * RB1, RB1), RB1)

    with jax.named_scope('blk0'):
        wq_copy(0).wait()
        in_order([wq_copy(j) for j in range(1, NWC)])
        qproj(ha_v[0], block(0), 0, 0, HPC // 2)
        x_copy(1).wait()
        ln1(1, hb_v, 0)
        qproj(ha_v[0], block(0), 0, HPC // 2, HPC)

    in_order([wr2_copy, wr_copy, wo_copy]
             + [cp for h in range(NS - UNROLL) for cp in kv_copies(h, h)] + [wg_copy, wu_copy, wd_copy])

    def pro_body(j, carry):
        more = 2 * j + 2 < NB1
        nxt = jnp.minimum(2 * j + 2, NB1 - 1)

        @pl.when(more)
        def _():
            x_copy(nxt).wait()

        ln1(nxt, ha_v, j + 1)
        qproj(hb_v[j], block(2 * j + 1), 0)

        @pl.when(more)
        def _():
            x_copy(nxt + 1).wait()
            ln1(nxt + 1, hb_v, j + 1)
            qproj(ha_v[j + 1], block(nxt), 0)
        return carry

    with jax.named_scope('pro'):
        lax.fori_loop(0, NB1 // 2, pro_body, 0)

    def qproj_body(j, carry):
        wq_copy(j).wait()
        h = jnp.concatenate([t for i in range(NB1 // 2) for t in (ha_v[i], hb_v[i])], axis=0)
        qproj(h, pl.ds(0, S), j)
        return carry

    with jax.named_scope('qproj'):
        lax.fori_loop(1, NWC, qproj_body, 0)
    with jax.named_scope('modrest'):
        wr2_copy.wait()
        mod_v[:, 2 * D:] = _dot(silu_c(), wm_v[:, 2 * D:6 * D])[0:8]

    def heads_step(g):
        h0 = g * UNROLL
        base = (g & 1) * UNROLL

        @pl.when(h0 + UNROLL < H)
        def _():
            for u in range(UNROLL):
                for cp in kv_copies(h0 + UNROLL + u, UNROLL - base + u):
                    cp.start()

        for u in range(UNROLL):
            for cp in kv_copies(h0 + u, base + u):
                cp.wait()
        return h0, base

    def fast_body(g, bad):
        h0, base = heads_step(g)
        for u in range(UNROLL):
            bad = bad + _attn_head_fast(q_v.at[h0 + u], k_v.at[base + u], v_v.at[base + u], o_v.at[h0 + u])
        return bad

    def exact_body(h, carry):
        slot = h & 1

        @pl.when(h + 1 < H)
        def _():
            for cp in kv_copies(h + 1, 1 - slot):
                cp.start()

        for cp in kv_copies(h, slot):
            cp.wait()
        _attn_head_exact(q_v.at[h], k_v.at[slot], v_v.at[slot], o_v.at[h])
        return carry

    with jax.named_scope('attn'):
        bad = lax.fori_loop(0, H // UNROLL, fast_body, jnp.full((8, DH), 0.0 if FAST else 1.0, F32))
    n_bad = jnp.sum(jnp.where(bad == 0.0, 0, 1))

    @pl.when(n_bad > 0)
    def _():
        for cp in kv_copies(0, 0):
            cp.start()
        lax.fori_loop(0, H, exact_body, 0)

    wr_copy.wait()
    wo_copy.wait()
    wr = jnp.concatenate([wr_v[j:j + 1, :] for j in range(D // 128)], axis=1).astype(F32)
    sub8 = lax.broadcasted_iota(I32, (8, DH), 0)

    def oproj(i, dst):
        rows = pl.ds(pl.multiple_of(i * RB3, RB3), RB3)
        o = jnp.concatenate([o_v[hd, rows, :] for hd in range(H)], axis=1)
        dst[...] = _dot(o, wo_v[...])

    def finish(i, src, top, pieces):
        t1, i1, t2, i2 = top
        live = i >= 0
        base = jnp.maximum(i, 0) * RB3
        dep = None
        off = 0
        for n in _pieces(RB3, pieces):
            rows = pl.ds(pl.multiple_of(base + off, 8), n)
            x1 = x_v[rows, :].astype(F32) + mod(2) * src[off:off + n, :]
            xn, _ = layernorm(x1, dep)
            h2 = (xn * (1.0 + mod(4)) + mod(3)).astype(BF16)
            y_v[rows, D:2 * D] = h2
            h2 = h2.astype(F32)
            r = jnp.sum(h2 * wr, axis=1, keepdims=True)
            y_v[rows, 0:D] = (x1 + mod(5) * (h2 + h2 * 0.0)).astype(BF16)
            dep = mark(r)
            r = jnp.where(live, r, -jnp.inf)
            for t in range(n // 8):
                rt = jnp.broadcast_to(r[t * 8:(t + 1) * 8], (8, DH))
                idx = sub8 + (base + off + t * 8)
                g1 = rt > t1
                g2 = rt > t2
                t2 = jnp.where(g1, t1, jnp.where(g2, rt, t2))
                i2 = jnp.where(g1, i1, jnp.where(g2, idx, i2))
                t1 = jnp.where(g1, rt, t1)
                i1 = jnp.where(g1, idx, i1)
            off += n
        return t1, i1, t2, i2

    def oproj_body(j, top):
        top = finish(2 * j - 1, att_b, top, NP3)
        oproj(2 * j, att_a)

        @pl.when(j > 0)
        def _():
            out_copy(2 * j - 1).start()

        top = finish(2 * j, att_a, top, NP3)
        oproj(2 * j + 1, att_b)
        out_copy(2 * j).start()
        return top

    ninf = jnp.full((8, DH), -jnp.inf, F32)
    none = jnp.full((8, DH), S, I32)
    with jax.named_scope('oproj'):
        top = lax.fori_loop(0, NB3 // 2, oproj_body, (ninf, none, ninf, none))
    with jax.named_scope('fin'):
        t1, i1, t2, i2 = finish(NB3 - 1, att_b, top, 1)
    out_copy(NB3 - 1).start()

    m1 = jnp.max(t1, axis=0, keepdims=True)
    a1 = jnp.min(jnp.where(t1 == m1, i1, S), axis=0, keepdims=True)
    won = i1 == a1
    t1b = jnp.where(won, t2, t1)
    i1b = jnp.where(won, i2, i1)
    m2 = jnp.max(t1b, axis=0, keepdims=True)
    a2 = jnp.min(jnp.where(t1b == m2, i1b, S), axis=0, keepdims=True)
    idx1 = jnp.minimum(a1[0, 0], S - 1)
    idx2 = jnp.minimum(a2[0, 0], S - 1)

    def slab(idx):
        return pl.ds(pl.multiple_of(idx & ~15, 16), 16)

    sub = lax.broadcasted_iota(I32, (16, D), 0)

    def pick_row(idx):
        rows = y_v[slab(idx), D:2 * D].astype(F32)
        return jnp.sum(jnp.where(sub == (idx & 15), rows, 0.0), axis=0, keepdims=True)

    xs = jnp.where(sub == 0, pick_row(idx1), jnp.where(sub == 1, pick_row(idx2), 0.0)).astype(BF16)

    with jax.named_scope('ffn'):
        wg_copy.wait()
        wu_copy.wait()
        wd_copy.wait()
        g = _dot(xs, wg_v[...])
        u = _dot(xs, wu_v[...])
        a = (g * jax.nn.sigmoid(g) * u).astype(BF16)
        y = _dot(a, wd_v[:, 0:D])
    gb = mod(5)
    d1 = gb * (y[0:1] * jax.nn.sigmoid(m1[:, 0:1]))
    d2 = gb * (y[1:2] * jax.nn.sigmoid(m2[:, 0:1]))

    for i in range(NB3):
        out_copy(i).wait()

    for idx, d in ((idx1, d1), (idx2, d2)):
        rows = slab(idx)
        y_v[rows, 0:D] = (y_v[rows, 0:D].astype(F32) + jnp.where(sub == (idx & 15), d, 0.0)).astype(BF16)
    patch = [pltpu.make_async_copy(y_v.at[slab(idx), 0:D], out_hbm.at[0, slab(idx), :], misc_sem.at[2 + n])
             for n, idx in enumerate((idx1, idx2))]
    patch[0].start()

    @pl.when((idx1 >> 4) != (idx2 >> 4))
    def _():
        patch[1].start()
        patch[1].wait()

    patch[0].wait()


@jax.jit
def pallas_adaLN_cond__mha_block_cached__moe_arch_mod__prompt_kernel(
    A_x: jax.Array,
    A_k_cache: jax.Array,
    A_v_cache: jax.Array,
    A_wq: jax.Array,
    A_wo: jax.Array,
    B_x: jax.Array,
    B_w_r: jax.Array,
    B_w_gate: jax.Array,
    B_w_up: jax.Array,
    B_w_down: jax.Array,
    c: jax.Array,
    w_mod: jax.Array,
):
    del B_x
    any_spec = pl.BlockSpec(memory_space=pl.ANY)
    NS = 2 * UNROLL
    NB1 = S // RB1
    scratch = [
        pltpu.VMEM((S, D), BF16),
        pltpu.VMEM((NB1 // 2 + 1, RB1, D), BF16),
        pltpu.VMEM((NB1 // 2, RB1, D), BF16),
        pltpu.VMEM((H, S, DH), BF16),
        pltpu.VMEM((H, S, DH), BF16),
        pltpu.VMEM((NS, S, DH), BF16),
        pltpu.VMEM((NS, S, DH), BF16),
        pltpu.VMEM((H * DH // WC, D, WC), BF16),
        pltpu.VMEM((H * DH, D), BF16),
        pltpu.VMEM((D, 6 * D + PADM), BF16),
        pltpu.VMEM((D, F), BF16),
        pltpu.VMEM((D, F), BF16),
        pltpu.VMEM((F, D + PAD), BF16),
        pltpu.VMEM((1, D), BF16),
        pltpu.VMEM((D // 128, 128), BF16),
        pltpu.VMEM((8, 6 * D), F32),
        pltpu.VMEM((RB3, D), F32),
        pltpu.VMEM((RB3, D), F32),
        pltpu.VMEM((S, 2 * D), BF16),
        pltpu.VMEM((8, DH), I32),
        pltpu.SemaphoreType.DMA((2, NS)),
        pltpu.SemaphoreType.DMA((S // RB1,)),
        pltpu.SemaphoreType.DMA((NKC,)),
        pltpu.SemaphoreType.DMA((H * DH // WC,)),
        pltpu.SemaphoreType.DMA((4,)),
        pltpu.SemaphoreType.DMA((5,)),
        pltpu.SemaphoreType.DMA((S // RB3,)),
        pltpu.SemaphoreType.REGULAR,
    ]
    return pl.pallas_call(
        _kernel,
        out_shape=jax.ShapeDtypeStruct((1, S, D), BF16),
        in_specs=[any_spec] * 11,
        out_specs=any_spec,
        scratch_shapes=scratch,
        compiler_params=pltpu.CompilerParams(vmem_limit_bytes=VMEM_MB * 1024 * 1024, disable_bounds_checks=NOBC),
    )(A_x, A_k_cache, A_v_cache, A_wq, A_wo, B_w_r.reshape(D // 128, 128), B_w_gate, B_w_up, B_w_down,
      c, w_mod)
```

```python
import functools
import math

import jax
import jax.numpy as jnp
from jax import lax
import jax.experimental.pallas as pl
import jax.experimental.pallas.tpu as pltpu

S = 2048
D = 1024
H = 32
DH = 128
F = 3584
BQ = 512
BK = 1024
RB1 = 256
NP1 = 7
WC = 512
NKC = 2
RB3 = 256
NP3 = 32
UNROLL = 2
EPS = 1e-5
Q_SCALE = (DH ** -0.5) * math.log2(math.e)
L_MIN = 2.0 ** -30
L_MAX = 2.0 ** 64
VMEM_MB = 122
NOBC = True
LINK = 1
NPB = 7
XWAIT = [1, 2, 3, 7, 7, 7, 7, 7]
NP0 = 4
FAST = True
PAD = 128
PADM = 128

BF16 = jnp.bfloat16
F32 = jnp.float32
I32 = jnp.int32
NT = (((1,), (1,)), ((), ()))


def _pieces(rows, n):
    unit = 16 if rows // 16 >= n else 8
    units = rows // unit
    return [unit * (units // n + (1 if c < units % n else 0)) for c in range(n)]


def _dot(a, b):
    return jnp.dot(a, b, preferred_element_type=F32)


def _qk(q, k):
    return lax.dot_general(q, k, NT, preferred_element_type=F32)


def _attn_head_fast(q_ref, k_ref, v_ref, o_ref, hook=None):
    bad = jnp.zeros((8, DH), F32)
    for i in range(S // BQ):
        rows = slice(i * BQ, (i + 1) * BQ)
        q = q_ref[rows, :]
        if hook is not None:
            q = hook(q)
        acc = l = None
        for a in range(0, S, BK):
            p = jnp.exp2(_qk(q, k_ref[a:a + BK, :]))
            for t in range(BK // DH):
                pt = p[:, t * DH:(t + 1) * DH]
                l = pt if l is None else l + pt
            pv = _dot(p.astype(BF16), v_ref[a:a + BK, :])
            acc = pv if acc is None else acc + pv
        l = jnp.sum(l, axis=1, keepdims=True)
        o = acc * jnp.where((l >= L_MIN) & (l <= L_MAX), 1.0 / l, jnp.nan)
        o_ref[rows, :] = o.astype(BF16)
        z = o * 0.0
        for t in range(BQ // 8):
            bad = bad + z[t * 8:(t + 1) * 8]
    return bad


def _attn_head_exact(q_ref, k_ref, v_ref, o_ref):
    def body(i, carry):
        rows = pl.ds(pl.multiple_of(i * BQ, BQ), BQ)
        s = _qk(q_ref[rows, :], k_ref[...])
        p = jnp.exp2(s - jnp.max(s, axis=1, keepdims=True))
        l = jnp.sum(p, axis=1, keepdims=True)
        o_ref[rows, :] = (_dot(p.astype(BF16), v_ref[...]) / l).astype(BF16)
        return carry
    lax.fori_loop(0, S // BQ, body, 0)


def _kernel(x_hbm, k_hbm, v_hbm, wq_hbm, wo_hbm, wr_hbm, wg_hbm, wu_hbm, wd_hbm, c_hbm, wm_hbm,
            out_hbm,
            x_v, h_v, q_v, o_v, k_v, v_v, wq_v, wo_v, wm_v, wg_v, wu_v, wd_v, c_v, wr_v, mod_v, mod2_v, scol_v,
            att_a, att_b, y_v, zero_v,
            kv_sem, x_sem, wa_sem, wq_sem, w_sem, misc_sem, out_sem, fence_sem):
    NB1 = S // RB1
    NB3 = S // RB3
    NWC = H * DH // WC
    HPC = WC // DH
    NS = 2 * UNROLL
    KC = D // NKC

    def kv_copies(h, slot):
        return (
            pltpu.make_async_copy(k_hbm.at[0, h], k_v.at[slot], kv_sem.at[0, slot]),
            pltpu.make_async_copy(v_hbm.at[0, h], v_v.at[slot], kv_sem.at[1, slot]),
        )

    def x_copy(i):
        rows = pl.ds(pl.multiple_of(i * RB1, RB1), RB1)
        return pltpu.make_async_copy(x_hbm.at[0, rows, :], x_v.at[rows, :], x_sem.at[i])

    def wa_copy(j):
        rows = pl.ds(j * KC, KC)
        return pltpu.make_async_copy(wm_hbm.at[rows, 0:2 * D], wm_v.at[rows, 0:2 * D], wa_sem.at[j])

    def wq_copy(j):
        cols = pl.ds(pl.multiple_of(j * WC, WC), WC)
        return pltpu.make_async_copy(wq_hbm.at[:, cols], wq_v.at[j], wq_sem.at[j])

    def out_copy(i):
        rows = pl.ds(pl.multiple_of(i * RB3, RB3), RB3)
        return pltpu.make_async_copy(y_v.at[rows, 0:D], out_hbm.at[0, rows, :], out_sem.at[i])

    c_copy = pltpu.make_async_copy(c_hbm, c_v, misc_sem.at[0])
    wr2_copy = pltpu.make_async_copy(wm_hbm.at[:, 2 * D:6 * D], wm_v.at[:, 2 * D:6 * D], misc_sem.at[4])
    wr_copy = pltpu.make_async_copy(wr_hbm, wr_v, misc_sem.at[1])
    wo_copy = pltpu.make_async_copy(wo_hbm, wo_v, w_sem.at[0])
    wg_copy = pltpu.make_async_copy(wg_hbm, wg_v, w_sem.at[1])
    wu_copy = pltpu.make_async_copy(wu_hbm, wu_v, w_sem.at[2])
    wd_copy = pltpu.make_async_copy(wd_hbm, wd_v.at[:, 0:D], w_sem.at[3])

    def after(val, dep):
        if dep is None:
            return val
        dep = jnp.tile(dep, (val.shape[0] // 8, 1))
        return lax.bitcast_convert_type(lax.bitcast_convert_type(val, I32) | dep, F32)

    def mark(val):
        return lax.bitcast_convert_type(val[val.shape[0] - 8:], I32) & zero_v[:, 0:1]

    def layernorm(x, dep, n=None):
        m = after(jnp.mean(x, axis=1, keepdims=True), dep)
        xc = x - m
        v = jnp.mean(xc * xc, axis=1, keepdims=True)
        return xc * lax.rsqrt(v + EPS), v

    def mod(j):
        if j < 2:
            return mod_v[0:1, j * D:(j + 1) * D]
        per = D * H // (4 * D * UNROLL)
        return jnp.concatenate([mod2_v[(j - 2) * per + t][0:1, :] for t in range(per)], axis=1)

    def silu_c():
        c32 = c_v[...].astype(F32)
        return jnp.broadcast_to((c32 * jax.nn.sigmoid(c32)).astype(BF16), (16, D))

    def in_order(copies):
        for cp in copies:
            cp.start()
            pl.semaphore_signal(fence_sem, 1)
            pl.semaphore_wait(fence_sem, 1)

    in_order([c_copy, x_copy(0)] + [wa_copy(j) for j in range(NKC)] + [wq_copy(0)]
             + [x_copy(i) for i in range(1, NB1)])
    zero_v[...] = jnp.zeros((8, DH), I32)
    att_b[...] = jnp.zeros((RB3, D), F32)

    with jax.named_scope('c'):
        c_copy.wait()
        sc = silu_c()
    with jax.named_scope('x0'):
        x_copy(0).wait()
        xn0, _ = layernorm(x_v[0:RB1, :].astype(F32), None)
    with jax.named_scope('moda'):
        acc = None
        for j in range(NKC):
            wa_copy(j).wait()
            part = _dot(sc[:, j * KC:(j + 1) * KC], wm_v[j * KC:(j + 1) * KC, 0:2 * D])
            acc = part if acc is None else acc + part
        mod_v[:, 0:2 * D] = acc[0:8]
        h_v[0:RB1, :] = (xn0 * (1.0 + acc[0:1, D:2 * D]) + acc[0:1, 0:D]).astype(BF16)

    def ln1(i, pieces):
        dep = None
        off = i * RB1
        for n in _pieces(RB1, pieces):
            xn, v = layernorm(x_v[off:off + n, :].astype(F32), dep)
            h_v[off:off + n, :] = (xn * (1.0 + mod(1)) + mod(0)).astype(BF16)
            dep = mark(v) if LINK else mark(xn)
            off += n

    def qproj(rows, j, t0=0, t1=HPC):
        q = _dot(h_v[rows, :], wq_v[j, :, t0 * DH:t1 * DH])
        for t in range(t0, t1):
            q_v[j * HPC + t, rows, :] = (q[:, (t - t0) * DH:(t - t0 + 1) * DH] * Q_SCALE).astype(BF16)

    with jax.named_scope('blk0'):
        wq_copy(0).wait()
        in_order([wq_copy(j) for j in range(1, NWC)])
        qproj(slice(0, RB1), 0, 0, HPC // 2)
        x_copy(1).wait()
        ln1(1, NP0)
        qproj(slice(0, RB1), 0, HPC // 2, HPC)

    in_order([wr2_copy, wr_copy, wo_copy]
             + [cp for h in range(NS - UNROLL) for cp in kv_copies(h, h)] + [wg_copy, wu_copy, wd_copy])

    with jax.named_scope('pro'):
        arrived = 2
        for i in range(1, NB1):
            while arrived <= min(XWAIT[i], NB1 - 1):
                x_copy(arrived).wait()
                arrived += 1
            if i + 1 < NB1:
                ln1(i + 1, NP1 if XWAIT[i] > XWAIT[i - 1] else NPB)
            qproj(slice(i * RB1, (i + 1) * RB1), 0)

    def qproj_body(j, carry):
        wq_copy(j).wait()
        qproj(slice(0, S), j)
        return carry

    with jax.named_scope('qproj'):
        lax.fori_loop(1, NWC, qproj_body, 0)

    wr2_copy.wait()
    c32 = c_v[...].astype(F32)
    scol_v[...] = jnp.broadcast_to((c32 * jax.nn.sigmoid(c32)).astype(BF16).astype(F32), (DH, D)).T
    MC = 4 * D * UNROLL // H

    def mod_cols(g):
        cols = pl.ds(pl.multiple_of(2 * D + g * MC, DH), MC)
        n = D // (UNROLL * S // BQ)
        state = [0, None]

        def step(q):
            r0 = state[0]
            sc_t = jnp.concatenate([scol_v[r0:r0 + n, :]] * (MC // DH), axis=1)
            prod = wm_v[r0:r0 + n, cols].astype(F32) * sc_t
            acc = state[1]
            for t in range(n // 8):
                acc = prod[t * 8:(t + 1) * 8] if acc is None else acc + prod[t * 8:(t + 1) * 8]
            state[0], state[1] = r0 + n, acc
            dep = lax.bitcast_convert_type(acc[:, 0:DH], I32) & zero_v[...]
            q0 = pltpu.bitcast(pltpu.bitcast(q[0:16], I32) | dep, BF16)
            return jnp.concatenate([q0, q[16:]], axis=0)

        def done():
            mod2_v[g] = jnp.broadcast_to(jnp.sum(state[1], axis=0, keepdims=True), (8, MC))

        return step, done

    def heads_step(g):
        h0 = g * UNROLL
        base = (g & 1) * UNROLL

        @pl.when(h0 + UNROLL < H)
        def _():
            for u in range(UNROLL):
                for cp in kv_copies(h0 + UNROLL + u, UNROLL - base + u):
                    cp.start()

        for u in range(UNROLL):
            for cp in kv_copies(h0 + u, base + u):
                cp.wait()
        return h0, base

    def fast_body(g, bad):
        h0, base = heads_step(g)
        step, done = mod_cols(g)
        for u in range(UNROLL):
            bad = bad + _attn_head_fast(q_v.at[h0 + u], k_v.at[base + u], v_v.at[base + u], o_v.at[h0 + u], step)
        done()
        return bad

    def exact_body(h, carry):
        slot = h & 1

        @pl.when(h + 1 < H)
        def _():
            for cp in kv_copies(h + 1, 1 - slot):
                cp.start()

        for cp in kv_copies(h, slot):
            cp.wait()
        _attn_head_exact(q_v.at[h], k_v.at[slot], v_v.at[slot], o_v.at[h])
        return carry

    with jax.named_scope('attn'):
        bad = lax.fori_loop(0, H // UNROLL, fast_body, jnp.full((8, DH), 0.0 if FAST else 1.0, F32))
    n_bad = jnp.sum(jnp.where(bad == 0.0, 0, 1))

    @pl.when(n_bad > 0)
    def _():
        for cp in kv_copies(0, 0):
            cp.start()
        lax.fori_loop(0, H, exact_body, 0)

    wr_copy.wait()
    wo_copy.wait()
    wr = jnp.concatenate([wr_v[j:j + 1, :] for j in range(D // 128)], axis=1).astype(F32)
    sub8 = lax.broadcasted_iota(I32, (8, DH), 0)

    def oproj(i, dst):
        rows = pl.ds(pl.multiple_of(i * RB3, RB3), RB3)
        o = jnp.concatenate([o_v[hd, rows, :] for hd in range(H)], axis=1)
        dst[...] = _dot(o, wo_v[...])

    def finish(i, src, top, pieces):
        t1, i1, t2, i2 = top
        live = i >= 0
        base = jnp.maximum(i, 0) * RB3
        dep = None
        off = 0
        for n in _pieces(RB3, pieces):
            rows = pl.ds(pl.multiple_of(base + off, 8), n)
            x1 = x_v[rows, :].astype(F32) + mod(2) * src[off:off + n, :]
            xn, _ = layernorm(x1, dep)
            h2 = (xn * (1.0 + mod(4)) + mod(3)).astype(BF16)
            y_v[rows, D:2 * D] = h2
            h2 = h2.astype(F32)
            r = jnp.sum(h2 * wr, axis=1, keepdims=True)
            y_v[rows, 0:D] = (x1 + mod(5) * (h2 + h2 * 0.0)).astype(BF16)
            dep = mark(r)
            r = jnp.where(live, r, -jnp.inf)
            for t in range(n // 8):
                rt = jnp.broadcast_to(r[t * 8:(t + 1) * 8], (8, DH))
                idx = sub8 + (base + off + t * 8)
                g1 = rt > t1
                g2 = rt > t2
                t2 = jnp.where(g1, t1, jnp.where(g2, rt, t2))
                i2 = jnp.where(g1, i1, jnp.where(g2, idx, i2))
                t1 = jnp.where(g1, rt, t1)
                i1 = jnp.where(g1, idx, i1)
            off += n
        return t1, i1, t2, i2

    def oproj_body(j, top):
        top = finish(2 * j - 1, att_b, top, NP3)
        oproj(2 * j, att_a)

        @pl.when(j > 0)
        def _():
            out_copy(2 * j - 1).start()

        top = finish(2 * j, att_a, top, NP3)
        oproj(2 * j + 1, att_b)
        out_copy(2 * j).start()
        return top

    ninf = jnp.full((8, DH), -jnp.inf, F32)
    none = jnp.full((8, DH), S, I32)
    with jax.named_scope('oproj'):
        top = lax.fori_loop(0, NB3 // 2, oproj_body, (ninf, none, ninf, none))
    with jax.named_scope('fin'):
        t1, i1, t2, i2 = finish(NB3 - 1, att_b, top, 1)
    out_copy(NB3 - 1).start()

    m1 = jnp.max(t1, axis=0, keepdims=True)
    a1 = jnp.min(jnp.where(t1 == m1, i1, S), axis=0, keepdims=True)
    won = i1 == a1
    t1b = jnp.where(won, t2, t1)
    i1b = jnp.where(won, i2, i1)
    m2 = jnp.max(t1b, axis=0, keepdims=True)
    a2 = jnp.min(jnp.where(t1b == m2, i1b, S), axis=0, keepdims=True)
    idx1 = jnp.minimum(a1[0, 0], S - 1)
    idx2 = jnp.minimum(a2[0, 0], S - 1)

    def slab(idx):
        return pl.ds(pl.multiple_of(idx & ~15, 16), 16)

    sub = lax.broadcasted_iota(I32, (16, D), 0)

    def pick_row(idx):
        rows = y_v[slab(idx), D:2 * D].astype(F32)
        return jnp.sum(jnp.where(sub == (idx & 15), rows, 0.0), axis=0, keepdims=True)

    xs = jnp.where(sub == 0, pick_row(idx1), jnp.where(sub == 1, pick_row(idx2), 0.0)).astype(BF16)

    with jax.named_scope('ffn'):
        wg_copy.wait()
        wu_copy.wait()
        wd_copy.wait()
        g = _dot(xs, wg_v[...])
        u = _dot(xs, wu_v[...])
        a = (g * jax.nn.sigmoid(g) * u).astype(BF16)
        y = _dot(a, wd_v[:, 0:D])
    gb = mod(5)
    d1 = gb * (y[0:1] * jax.nn.sigmoid(m1[:, 0:1]))
    d2 = gb * (y[1:2] * jax.nn.sigmoid(m2[:, 0:1]))

    for i in range(NB3):
        out_copy(i).wait()

    for idx, d in ((idx1, d1), (idx2, d2)):
        rows = slab(idx)
        y_v[rows, 0:D] = (y_v[rows, 0:D].astype(F32) + jnp.where(sub == (idx & 15), d, 0.0)).astype(BF16)
    patch = [pltpu.make_async_copy(y_v.at[slab(idx), 0:D], out_hbm.at[0, slab(idx), :], misc_sem.at[2 + n])
             for n, idx in enumerate((idx1, idx2))]
    patch[0].start()

    @pl.when((idx1 >> 4) != (idx2 >> 4))
    def _():
        patch[1].start()
        patch[1].wait()

    patch[0].wait()


@jax.jit
def pallas_adaLN_cond__mha_block_cached__moe_arch_mod__prompt_kernel(
    A_x: jax.Array,
    A_k_cache: jax.Array,
    A_v_cache: jax.Array,
    A_wq: jax.Array,
    A_wo: jax.Array,
    B_x: jax.Array,
    B_w_r: jax.Array,
    B_w_gate: jax.Array,
    B_w_up: jax.Array,
    B_w_down: jax.Array,
    c: jax.Array,
    w_mod: jax.Array,
):
    del B_x
    any_spec = pl.BlockSpec(memory_space=pl.ANY)
    NS = 2 * UNROLL
    NB1 = S // RB1
    scratch = [
        pltpu.VMEM((S, D), BF16),
        pltpu.VMEM((S, D), BF16),
        pltpu.VMEM((H, S, DH), BF16),
        pltpu.VMEM((H, S, DH), BF16),
        pltpu.VMEM((NS, S, DH), BF16),
        pltpu.VMEM((NS, S, DH), BF16),
        pltpu.VMEM((H * DH // WC, D, WC), BF16),
        pltpu.VMEM((H * DH, D), BF16),
        pltpu.VMEM((D, 6 * D + PADM), BF16),
        pltpu.VMEM((D, F), BF16),
        pltpu.VMEM((D, F), BF16),
        pltpu.VMEM((F, D + PAD), BF16),
        pltpu.VMEM((1, D), BF16),
        pltpu.VMEM((D // 128, 128), BF16),
        pltpu.VMEM((8, 2 * D), F32),
        pltpu.VMEM((H // UNROLL, 8, 4 * D * UNROLL // H), F32),
        pltpu.VMEM((D, DH), F32),
        pltpu.VMEM((RB3, D), F32),
        pltpu.VMEM((RB3, D), F32),
        pltpu.VMEM((S, 2 * D), BF16),
        pltpu.VMEM((8, DH), I32),
        pltpu.SemaphoreType.DMA((2, NS)),
        pltpu.SemaphoreType.DMA((S // RB1,)),
        pltpu.SemaphoreType.DMA((NKC,)),
        pltpu.SemaphoreType.DMA((H * DH // WC,)),
        pltpu.SemaphoreType.DMA((4,)),
        pltpu.SemaphoreType.DMA((5,)),
        pltpu.SemaphoreType.DMA((S // RB3,)),
        pltpu.SemaphoreType.REGULAR,
    ]
    return pl.pallas_call(
        _kernel,
        out_shape=jax.ShapeDtypeStruct((1, S, D), BF16),
        in_specs=[any_spec] * 11,
        out_specs=any_spec,
        scratch_shapes=scratch,
        compiler_params=pltpu.CompilerParams(vmem_limit_bytes=VMEM_MB * 1024 * 1024, disable_bounds_checks=NOBC),
    )(A_x, A_k_cache, A_v_cache, A_wq, A_wo, B_w_r.reshape(D // 128, 128), B_w_gate, B_w_up, B_w_down,
      c, w_mod)
```

```python
import functools
import math

import jax
import jax.numpy as jnp
from jax import lax
import jax.experimental.pallas as pl
import jax.experimental.pallas.tpu as pltpu

S = 2048
D = 1024
H = 32
DH = 128
F = 3584
BQ = 512
BK = 1024
RB1 = 256
NP1 = 7
WC = 512
NKC = 2
RB3 = 256
NP3 = 32
UNROLL = 2
EPS = 1e-5
Q_SCALE = (DH ** -0.5) * math.log2(math.e)
L_MIN = 2.0 ** -30
L_MAX = 2.0 ** 64
VMEM_MB = 122
NOBC = True
LINK = 1
TAILDMA = True
NPB = 7
XWAIT = [1, 2, 3, 7, 7, 7, 7, 7]
NP0 = 4
FAST = True
PAD = 128
PADM = 128

BF16 = jnp.bfloat16
F32 = jnp.float32
I32 = jnp.int32
NT = (((1,), (1,)), ((), ()))


def _pieces(rows, n):
    unit = 16 if rows // 16 >= n else 8
    units = rows // unit
    return [unit * (units // n + (1 if c < units % n else 0)) for c in range(n)]


def _r16(a):
    return a.astype(BF16).astype(F32)


def _dot(a, b):
    return jnp.dot(a, b, preferred_element_type=F32)


def _qk(q, k):
    return lax.dot_general(q, k, NT, preferred_element_type=F32)


def _attn_head_fast(q_ref, k_ref, v_ref, o_ref, hook=None):
    bad = jnp.zeros((8, DH), F32)
    for i in range(S // BQ):
        rows = slice(i * BQ, (i + 1) * BQ)
        q = q_ref[rows, :]
        if hook is not None:
            q = hook(q)
        acc = l = None
        for a in range(0, S, BK):
            p = jnp.exp2(_qk(q, k_ref[a:a + BK, :]))
            for t in range(BK // DH):
                pt = p[:, t * DH:(t + 1) * DH]
                l = pt if l is None else l + pt
            pv = _dot(p.astype(BF16), v_ref[a:a + BK, :])
            acc = pv if acc is None else acc + pv
        l = jnp.sum(l, axis=1, keepdims=True)
        o = acc * jnp.where((l >= L_MIN) & (l <= L_MAX), 1.0 / l, jnp.nan)
        o_ref[rows, :] = o.astype(BF16)
        z = o * 0.0
        for t in range(BQ // 8):
            bad = bad + z[t * 8:(t + 1) * 8]
    return bad


def _attn_head_exact(q_ref, k_ref, v_ref, o_ref):
    def body(i, carry):
        rows = pl.ds(pl.multiple_of(i * BQ, BQ), BQ)
        s = _qk(q_ref[rows, :], k_ref[...])
        p = jnp.exp2(s - jnp.max(s, axis=1, keepdims=True))
        l = jnp.sum(p, axis=1, keepdims=True)
        o_ref[rows, :] = (_dot(p.astype(BF16), v_ref[...]) / l).astype(BF16)
        return carry
    lax.fori_loop(0, S // BQ, body, 0)


def _kernel(x_hbm, k_hbm, v_hbm, wq_hbm, wo_hbm, wr_hbm, wg_hbm, wu_hbm, wd_hbm, c_hbm, wm_hbm,
            out_hbm,
            x_v, h_v, q_v, o_v, k_v, v_v, wq_v, wo_v, wm_v, wg_v, wu_v, wd_v, c_v, wr_v, mod_v, mod2_v, scol_v,
            att_a, att_b, y_v, zero_v,
            kv_sem, x_sem, wa_sem, wq_sem, w_sem, misc_sem, out_sem, fence_sem):
    NB1 = S // RB1
    NB3 = S // RB3
    NWC = H * DH // WC
    HPC = WC // DH
    NS = 2 * UNROLL
    KC = D // NKC

    def kv_copies(h, slot):
        return (
            pltpu.make_async_copy(k_hbm.at[0, h], k_v.at[slot], kv_sem.at[0, slot]),
            pltpu.make_async_copy(v_hbm.at[0, h], v_v.at[slot], kv_sem.at[1, slot]),
        )

    def x_copy(i):
        rows = pl.ds(pl.multiple_of(i * RB1, RB1), RB1)
        return pltpu.make_async_copy(x_hbm.at[0, rows, :], x_v.at[rows, :], x_sem.at[i])

    def wa_copy(j):
        rows = pl.ds(j * KC, KC)
        return pltpu.make_async_copy(wm_hbm.at[rows, 0:2 * D], wm_v.at[rows, 0:2 * D], wa_sem.at[j])

    def wq_copy(j):
        cols = pl.ds(pl.multiple_of(j * WC, WC), WC)
        return pltpu.make_async_copy(wq_hbm.at[:, cols], wq_v.at[j], wq_sem.at[j])

    def out_copy(i):
        rows = pl.ds(pl.multiple_of(i * RB3, RB3), RB3)
        return pltpu.make_async_copy(y_v.at[rows, 0:D], out_hbm.at[0, rows, :], out_sem.at[i])

    c_copy = pltpu.make_async_copy(c_hbm, c_v, misc_sem.at[0])
    wr2_copy = pltpu.make_async_copy(wm_hbm.at[:, 2 * D:6 * D], wm_v.at[:, 2 * D:6 * D], misc_sem.at[4])
    wr_copy = pltpu.make_async_copy(wr_hbm, wr_v, misc_sem.at[1])
    wo_copy = pltpu.make_async_copy(wo_hbm, wo_v, w_sem.at[0])
    wg_copy = pltpu.make_async_copy(wg_hbm, wg_v, w_sem.at[1])
    wu_copy = pltpu.make_async_copy(wu_hbm, wu_v, w_sem.at[2])
    wd_copy = pltpu.make_async_copy(wd_hbm, wd_v.at[:, 0:D], w_sem.at[3])

    def after(val, dep):
        if dep is None:
            return val
        dep = jnp.tile(dep, (val.shape[0] // 8, 1))
        return lax.bitcast_convert_type(lax.bitcast_convert_type(val, I32) | dep, F32)

    def mark(val):
        return lax.bitcast_convert_type(val[val.shape[0] - 8:], I32) & zero_v[:, 0:1]

    def layernorm(x, dep, like_ref=False):
        m = after(jnp.mean(x, axis=1, keepdims=True), dep)
        xc = x - m
        v = jnp.mean(xc * xc, axis=1, keepdims=True)
        if like_ref:
            return xc * (1.0 / _r16(jnp.sqrt(_r16(_r16(v) + EPS)))), v
        return xc * lax.rsqrt(v + EPS), v

    def mod(j):
        if j < 2:
            return mod_v[0:1, j * D:(j + 1) * D]
        per = D * H // (4 * D * UNROLL)
        return jnp.concatenate([mod2_v[(j - 2) * per + t][0:1, :] for t in range(per)], axis=1)

    def silu_c():
        c32 = c_v[...].astype(F32)
        return jnp.broadcast_to((c32 * jax.nn.sigmoid(c32)).astype(BF16), (16, D))

    def in_order(copies):
        for cp in copies:
            cp.start()
            pl.semaphore_signal(fence_sem, 1)
            pl.semaphore_wait(fence_sem, 1)

    in_order([c_copy, x_copy(0)] + [wa_copy(j) for j in range(NKC)] + [wq_copy(0)]
             + [x_copy(i) for i in range(1, NB1)])
    zero_v[...] = jnp.zeros((8, DH), I32)
    att_b[...] = jnp.zeros((RB3, D), F32)

    with jax.named_scope('c'):
        c_copy.wait()
        sc = silu_c()
        scol_v[...] = jnp.broadcast_to(sc[0:1].astype(F32), (DH, D)).T
    with jax.named_scope('x0'):
        x_copy(0).wait()
        xn0, _ = layernorm(x_v[0:RB1, :].astype(F32), None)
    with jax.named_scope('moda'):
        acc = None
        for j in range(NKC):
            wa_copy(j).wait()
            part = _dot(sc[:, j * KC:(j + 1) * KC], wm_v[j * KC:(j + 1) * KC, 0:2 * D])
            acc = part if acc is None else acc + part
        mod_v[:, 0:2 * D] = acc[0:8]
        h_v[0:RB1, :] = (xn0 * (1.0 + acc[0:1, D:2 * D]) + acc[0:1, 0:D]).astype(BF16)

    def ln1(i, pieces):
        dep = None
        off = i * RB1
        for n in _pieces(RB1, pieces):
            xn, v = layernorm(x_v[off:off + n, :].astype(F32), dep)
            h_v[off:off + n, :] = (xn * (1.0 + mod(1)) + mod(0)).astype(BF16)
            dep = mark(v) if LINK else mark(xn)
            off += n

    def qproj(rows, j, t0=0, t1=HPC):
        q = _dot(h_v[rows, :], wq_v[j, :, t0 * DH:t1 * DH])
        for t in range(t0, t1):
            q_v[j * HPC + t, rows, :] = (q[:, (t - t0) * DH:(t - t0 + 1) * DH] * Q_SCALE).astype(BF16)

    with jax.named_scope('blk0'):
        wq_copy(0).wait()
        in_order([wq_copy(j) for j in range(1, NWC)])
        qproj(slice(0, RB1), 0, 0, HPC // 2)
        x_copy(1).wait()
        ln1(1, NP0)
        qproj(slice(0, RB1), 0, HPC // 2, HPC)

    in_order([wr2_copy, wr_copy, wo_copy]
             + [cp for h in range(NS if TAILDMA else UNROLL) for cp in kv_copies(h, h)] + [wg_copy, wu_copy, wd_copy])

    with jax.named_scope('pro'):
        arrived = 2
        for i in range(1, NB1):
            while arrived <= min(XWAIT[i], NB1 - 1):
                x_copy(arrived).wait()
                arrived += 1
            if i + 1 < NB1:
                ln1(i + 1, NP1 if XWAIT[i] > XWAIT[i - 1] else NPB)
            qproj(slice(i * RB1, (i + 1) * RB1), 0)

    def qproj_body(j, carry):
        wq_copy(j).wait()
        qproj(slice(0, S), j)
        return carry

    with jax.named_scope('qproj'):
        lax.fori_loop(1, NWC, qproj_body, 0)

    wr2_copy.wait()
    MC = 4 * D * UNROLL // H

    def mod_cols(g):
        cols = pl.ds(pl.multiple_of(2 * D + g * MC, DH), MC)
        n = D // (UNROLL * S // BQ)
        state = [0, None]

        def step(q):
            r0 = state[0]
            sc_t = jnp.concatenate([scol_v[r0:r0 + n, :]] * (MC // DH), axis=1)
            prod = wm_v[r0:r0 + n, cols].astype(F32) * sc_t
            acc = state[1]
            for t in range(n // 8):
                acc = prod[t * 8:(t + 1) * 8] if acc is None else acc + prod[t * 8:(t + 1) * 8]
            state[0], state[1] = r0 + n, acc
            dep = lax.bitcast_convert_type(acc[:, 0:DH], I32) & zero_v[...]
            q0 = pltpu.bitcast(pltpu.bitcast(q[0:16], I32) | dep, BF16)
            return jnp.concatenate([q0, q[16:]], axis=0)

        def done():
            mod2_v[g] = jnp.broadcast_to(jnp.sum(state[1], axis=0, keepdims=True), (8, MC))

        return step, done

    def heads_step(g):
        h0 = g * UNROLL
        base = (g & 1) * UNROLL

        @pl.when(h0 + UNROLL < H)
        def _():
            for u in range(UNROLL):
                for cp in kv_copies(h0 + UNROLL + u, UNROLL - base + u):
                    cp.start()

        for u in range(UNROLL):
            for cp in kv_copies(h0 + u, base + u):
                cp.wait()
        return h0, base

    def fast_body(g, bad):
        if not TAILDMA:
            h0, base = heads_step(g)
        else:
            h0 = g * UNROLL
            base = (g & 1) * UNROLL
        step, done = mod_cols(g)
        for u in range(UNROLL):
            bad = bad + _attn_head_fast(q_v.at[h0 + u], k_v.at[base + u], v_v.at[base + u], o_v.at[h0 + u], step)
        done()
        if TAILDMA:
            @pl.when(h0 + UNROLL < H)
            def _():
                for u in range(UNROLL):
                    for cp in kv_copies(h0 + UNROLL + u, UNROLL - base + u):
                        cp.wait()

            @pl.when(h0 + 2 * UNROLL < H)
            def _():
                for u in range(UNROLL):
                    for cp in kv_copies(h0 + 2 * UNROLL + u, base + u):
                        cp.start()
        return bad

    if TAILDMA:
        for u in range(UNROLL):
            for cp in kv_copies(u, u):
                cp.wait()

    def exact_body(h, carry):
        slot = h & 1

        @pl.when(h + 1 < H)
        def _():
            for cp in kv_copies(h + 1, 1 - slot):
                cp.start()

        for cp in kv_copies(h, slot):
            cp.wait()
        _attn_head_exact(q_v.at[h], k_v.at[slot], v_v.at[slot], o_v.at[h])
        return carry

    with jax.named_scope('attn'):
        bad = lax.fori_loop(0, H // UNROLL, fast_body, jnp.full((8, DH), 0.0 if FAST else 1.0, F32))
    n_bad = jnp.sum(jnp.where(bad == 0.0, 0, 1))

    @pl.when(n_bad > 0)
    def _():
        for cp in kv_copies(0, 0):
            cp.start()
        lax.fori_loop(0, H, exact_body, 0)

    wr_copy.wait()
    wo_copy.wait()
    wr = jnp.concatenate([wr_v[j:j + 1, :] for j in range(D // 128)], axis=1).astype(F32)
    scale_b = _r16(1.0 + mod(4))
    sub8 = lax.broadcasted_iota(I32, (8, DH), 0)

    def oproj(i, dst):
        rows = pl.ds(pl.multiple_of(i * RB3, RB3), RB3)
        o = jnp.concatenate([o_v[hd, rows, :] for hd in range(H)], axis=1)
        dst[...] = _dot(o, wo_v[...])

    def finish(i, src, top, pieces):
        t1, i1, t2, i2 = top
        live = i >= 0
        base = jnp.maximum(i, 0) * RB3
        dep = None
        off = 0
        for n in _pieces(RB3, pieces):
            rows = pl.ds(pl.multiple_of(base + off, 8), n)
            x1 = x_v[rows, :].astype(F32) + mod(2) * src[off:off + n, :]
            xn, _ = layernorm(x1, dep, True)
            h2 = xn * scale_b + mod(3)
            y_v[rows, D:2 * D] = h2.astype(BF16)
            r = _r16(jnp.sum(h2 * wr, axis=1, keepdims=True))
            y_v[rows, 0:D] = (x1 + mod(5) * (h2 + h2 * 0.0)).astype(BF16)
            dep = mark(r)
            r = jnp.where(live, r, -jnp.inf)
            for t in range(n // 8):
                rt = jnp.broadcast_to(r[t * 8:(t + 1) * 8], (8, DH))
                idx = sub8 + (base + off + t * 8)
                g1 = rt > t1
                g2 = rt > t2
                t2 = jnp.where(g1, t1, jnp.where(g2, rt, t2))
                i2 = jnp.where(g1, i1, jnp.where(g2, idx, i2))
                t1 = jnp.where(g1, rt, t1)
                i1 = jnp.where(g1, idx, i1)
            off += n
        return t1, i1, t2, i2

    def oproj_body(j, top):
        top = finish(2 * j - 1, att_b, top, NP3)
        oproj(2 * j, att_a)

        @pl.when(j > 0)
        def _():
            out_copy(2 * j - 1).start()

        top = finish(2 * j, att_a, top, NP3)
        oproj(2 * j + 1, att_b)
        out_copy(2 * j).start()
        return top

    ninf = jnp.full((8, DH), -jnp.inf, F32)
    none = jnp.full((8, DH), S, I32)
    with jax.named_scope('oproj'):
        top = lax.fori_loop(0, NB3 // 2, oproj_body, (ninf, none, ninf, none))
    for i in range(NB3 - 1):
        out_copy(i).wait()
    wg_copy.wait()
    wu_copy.wait()
    wd_copy.wait()
    with jax.named_scope('fin'):
        t1, i1, t2, i2 = finish(NB3 - 1, att_b, top, 1)
    out_copy(NB3 - 1).start()

    m1 = jnp.max(t1, axis=0, keepdims=True)
    a1 = jnp.min(jnp.where(t1 == m1, i1, S), axis=0, keepdims=True)
    won = i1 == a1
    t1b = jnp.where(won, t2, t1)
    i1b = jnp.where(won, i2, i1)
    m2 = jnp.max(t1b, axis=0, keepdims=True)
    a2 = jnp.min(jnp.where(t1b == m2, i1b, S), axis=0, keepdims=True)
    idx1 = jnp.minimum(a1[0, 0], S - 1)
    idx2 = jnp.minimum(a2[0, 0], S - 1)

    def slab(idx):
        return pl.ds(pl.multiple_of(idx & ~15, 16), 16)

    sub = lax.broadcasted_iota(I32, (16, D), 0)

    def pick_row(idx):
        rows = y_v[slab(idx), D:2 * D].astype(F32)
        return jnp.sum(jnp.where(sub == (idx & 15), rows, 0.0), axis=0, keepdims=True)

    xs = jnp.where(sub == 0, pick_row(idx1), jnp.where(sub == 1, pick_row(idx2), 0.0)).astype(BF16)

    with jax.named_scope('ffn'):
        g = _dot(xs, wg_v[...])
        u = _dot(xs, wu_v[...])
        a = (g * jax.nn.sigmoid(g) * u).astype(BF16)
        y = _dot(a, wd_v[:, 0:D])
    gb = mod(5)
    d1 = gb * (y[0:1] * jax.nn.sigmoid(m1[:, 0:1]))
    d2 = gb * (y[1:2] * jax.nn.sigmoid(m2[:, 0:1]))

    out_copy(NB3 - 1).wait()

    for idx, d in ((idx1, d1), (idx2, d2)):
        rows = slab(idx)
        y_v[rows, 0:D] = (y_v[rows, 0:D].astype(F32) + jnp.where(sub == (idx & 15), d, 0.0)).astype(BF16)
    patch = [pltpu.make_async_copy(y_v.at[slab(idx), 0:D], out_hbm.at[0, slab(idx), :], misc_sem.at[2 + n])
             for n, idx in enumerate((idx1, idx2))]
    patch[0].start()

    @pl.when((idx1 >> 4) != (idx2 >> 4))
    def _():
        patch[1].start()
        patch[1].wait()

    patch[0].wait()


@jax.jit
def pallas_adaLN_cond__mha_block_cached__moe_arch_mod__prompt_kernel(
    A_x: jax.Array,
    A_k_cache: jax.Array,
    A_v_cache: jax.Array,
    A_wq: jax.Array,
    A_wo: jax.Array,
    B_x: jax.Array,
    B_w_r: jax.Array,
    B_w_gate: jax.Array,
    B_w_up: jax.Array,
    B_w_down: jax.Array,
    c: jax.Array,
    w_mod: jax.Array,
):
    del B_x
    any_spec = pl.BlockSpec(memory_space=pl.ANY)
    NS = 2 * UNROLL
    NB1 = S // RB1
    scratch = [
        pltpu.VMEM((S, D), BF16),
        pltpu.VMEM((S, D), BF16),
        pltpu.VMEM((H, S, DH), BF16),
        pltpu.VMEM((H, S, DH), BF16),
        pltpu.VMEM((NS, S, DH), BF16),
        pltpu.VMEM((NS, S, DH), BF16),
        pltpu.VMEM((H * DH // WC, D, WC), BF16),
        pltpu.VMEM((H * DH, D), BF16),
        pltpu.VMEM((D, 6 * D + PADM), BF16),
        pltpu.VMEM((D, F), BF16),
        pltpu.VMEM((D, F), BF16),
        pltpu.VMEM((F, D + PAD), BF16),
        pltpu.VMEM((1, D), BF16),
        pltpu.VMEM((D // 128, 128), BF16),
        pltpu.VMEM((8, 2 * D), F32),
        pltpu.VMEM((H // UNROLL, 8, 4 * D * UNROLL // H), F32),
        pltpu.VMEM((D, DH), F32),
        pltpu.VMEM((RB3, D), F32),
        pltpu.VMEM((RB3, D), F32),
        pltpu.VMEM((S, 2 * D), BF16),
        pltpu.VMEM((8, DH), I32),
        pltpu.SemaphoreType.DMA((2, NS)),
        pltpu.SemaphoreType.DMA((S // RB1,)),
        pltpu.SemaphoreType.DMA((NKC,)),
        pltpu.SemaphoreType.DMA((H * DH // WC,)),
        pltpu.SemaphoreType.DMA((4,)),
        pltpu.SemaphoreType.DMA((5,)),
        pltpu.SemaphoreType.DMA((S // RB3,)),
        pltpu.SemaphoreType.REGULAR,
    ]
    return pl.pallas_call(
        _kernel,
        out_shape=jax.ShapeDtypeStruct((1, S, D), BF16),
        in_specs=[any_spec] * 11,
        out_specs=any_spec,
        scratch_shapes=scratch,
        compiler_params=pltpu.CompilerParams(vmem_limit_bytes=VMEM_MB * 1024 * 1024, disable_bounds_checks=NOBC),
    )(A_x, A_k_cache, A_v_cache, A_wq, A_wo, B_w_r.reshape(D // 128, 128), B_w_gate, B_w_up, B_w_down,
      c, w_mod)
```

```python
import contextlib
import math

import jax
import jax.numpy as jnp
from jax import lax
import jax.experimental.pallas as pl
import jax.experimental.pallas.tpu as pltpu

S = 2048
D = 1024
H = 32
DH = 128
F = 3584
EPS = 1e-5

BQ = 512
BK = 1024
U = 2
BQX = 256
RB1 = 256
NP0 = 4
NP1 = 7
WC = 512
NKC = 2
RB3 = 256
NP3 = 32
PAD = 128
SCOPES = False

Q_SCALE = (DH ** -0.5) * math.log2(math.e)
L_MIN = 2.0 ** -30
L_MAX = 2.0 ** 64

NB1 = S // RB1
NB3 = S // RB3
NWC = H * DH // WC
HPC = WC // DH
KC = D // NKC
NG = H // U
MC = 4 * D // NG

BF16 = jnp.bfloat16
F32 = jnp.float32
I32 = jnp.int32
NT = (((1,), (1,)), ((), ()))


def _scope(name):
    return jax.named_scope(name) if SCOPES else contextlib.nullcontext()


def _dot(a, b):
    return jnp.dot(a, b, preferred_element_type=F32)


def _qk(q, k):
    return lax.dot_general(q, k, NT, preferred_element_type=F32)


def _r16(a):
    return a.astype(BF16).astype(F32)


def _pieces(rows, n):
    unit = 16 if rows // 16 >= n else 8
    units = rows // unit
    return [unit * (units // n + (1 if c < units % n else 0)) for c in range(n)]


def _attn_head_fast(q_ref, k_ref, v_ref, o_ref, hook):
    bad = jnp.zeros((8, DH), F32)
    for i in range(S // BQ):
        rows = slice(i * BQ, (i + 1) * BQ)
        q = hook(q_ref[rows, :])
        acc = l = None
        for a in range(0, S, BK):
            p = jnp.exp2(_qk(q, k_ref[a:a + BK, :]))
            for t in range(BK // DH):
                pt = p[:, t * DH:(t + 1) * DH]
                l = pt if l is None else l + pt
            pv = _dot(p.astype(BF16), v_ref[a:a + BK, :])
            acc = pv if acc is None else acc + pv
        l = jnp.sum(l, axis=1, keepdims=True)
        o = acc * jnp.where((l >= L_MIN) & (l <= L_MAX), 1.0 / l, jnp.nan)
        o_ref[rows, :] = o.astype(BF16)
        z = o * 0.0
        for t in range(BQ // 8):
            bad = bad + z[t * 8:(t + 1) * 8]
    return bad


def _attn_rows_exact(q_ref, k_ref, v_ref, o_ref, i):
    rows = pl.ds(pl.multiple_of(i * BQX, BQX), BQX)
    s = _qk(q_ref[rows, :], k_ref[...])
    p = jnp.exp2(s - jnp.max(s, axis=1, keepdims=True))
    l = jnp.sum(p, axis=1, keepdims=True)
    o_ref[rows, :] = (_dot(p.astype(BF16), v_ref[...]) / l).astype(BF16)


def _kernel(x_hbm, k_hbm, v_hbm, wq_hbm, wo_hbm, wr_hbm, wg_hbm, wu_hbm, wd_hbm, c_hbm, wm_hbm,
            out_hbm,
            x_v, h_v, q_v, o_v, k_v, v_v, wq_v, wo_v, wm_v, wg_v, wu_v, wd_v, c_v, wr_v,
            moda_v, modb_v, scol_v, att_a, att_b, y_v, zero_v,
            kv_sem, x_sem, wa_sem, wq_sem, w_sem, misc_sem, out_sem, fence_sem):

    def kv_copies(g, slot):
        heads = pl.ds(g * U, U)
        return (pltpu.make_async_copy(k_hbm.at[0, heads], k_v.at[slot], kv_sem.at[0, slot]),
                pltpu.make_async_copy(v_hbm.at[0, heads], v_v.at[slot], kv_sem.at[1, slot]))

    def x_copy(i):
        rows = pl.ds(i * RB1, RB1)
        return pltpu.make_async_copy(x_hbm.at[0, rows, :], x_v.at[rows, :], x_sem.at[i])

    def wa_copy(j):
        rows = pl.ds(j * KC, KC)
        return pltpu.make_async_copy(wm_hbm.at[rows, 0:2 * D], wm_v.at[rows, 0:2 * D], wa_sem.at[j])

    def wq_copy(j):
        cols = pl.ds(pl.multiple_of(j * WC, WC), WC)
        return pltpu.make_async_copy(wq_hbm.at[:, cols], wq_v.at[j], wq_sem.at[j])

    def out_copy(i):
        rows = pl.ds(pl.multiple_of(i * RB3, RB3), RB3)
        return pltpu.make_async_copy(y_v.at[rows, :], out_hbm.at[0, rows, :], out_sem.at[i])

    c_copy = pltpu.make_async_copy(c_hbm, c_v, misc_sem.at[0])
    wr_copy = pltpu.make_async_copy(wr_hbm, wr_v, misc_sem.at[1])
    wb_copy = pltpu.make_async_copy(wm_hbm.at[:, 2 * D:6 * D], wm_v.at[:, 2 * D:6 * D], misc_sem.at[2])
    wo_copy = pltpu.make_async_copy(wo_hbm, wo_v, w_sem.at[0])
    wg_copy = pltpu.make_async_copy(wg_hbm, wg_v, w_sem.at[1])
    wu_copy = pltpu.make_async_copy(wu_hbm, wu_v, w_sem.at[2])
    wd_copy = pltpu.make_async_copy(wd_hbm, wd_v.at[:, 0:D], w_sem.at[3])

    def in_order(copies):
        for cp in copies:
            cp.start()
            pl.semaphore_signal(fence_sem, 1)
            pl.semaphore_wait(fence_sem, 1)

    def mark(val):
        return lax.bitcast_convert_type(val[val.shape[0] - 8:], I32) & zero_v[:, 0:1]

    def after(val, dep):
        if dep is None:
            return val
        dep = jnp.tile(dep, (val.shape[0] // 8, 1))
        return lax.bitcast_convert_type(lax.bitcast_convert_type(val, I32) | dep, F32)

    def layernorm(x, dep, like_ref=False):
        m = after(jnp.mean(x, axis=1, keepdims=True), dep)
        xc = x - m
        v = jnp.mean(xc * xc, axis=1, keepdims=True)
        if like_ref:
            return xc * (1.0 / _r16(jnp.sqrt(_r16(_r16(v) + EPS)))), v
        return xc * lax.rsqrt(v + EPS), v

    in_order([c_copy, x_copy(0)] + [wa_copy(j) for j in range(NKC)] + [wq_copy(0)]
             + [x_copy(i) for i in range(1, NB1)])
    zero_v[...] = jnp.zeros((8, DH), I32)
    att_b[...] = jnp.zeros((RB3, D), F32)

    with _scope('moda'):
        c_copy.wait()
        c32 = c_v[...].astype(F32)
        sc = jnp.broadcast_to((c32 * jax.nn.sigmoid(c32)).astype(BF16), (16, D))
        scol_v[...] = jnp.broadcast_to(sc[0:1].astype(F32), (DH, D)).T
        x_copy(0).wait()
        xn0, _ = layernorm(x_v[0:RB1, :].astype(F32), None)
        acc = None
        for j in range(NKC):
            wa_copy(j).wait()
            part = _dot(sc[:, j * KC:(j + 1) * KC], wm_v[j * KC:(j + 1) * KC, 0:2 * D])
            acc = part if acc is None else acc + part
        moda_v[...] = acc[0:8]
        h_v[0:RB1, :] = (xn0 * (1.0 + acc[0:1, D:2 * D]) + acc[0:1, 0:D]).astype(BF16)

    def ln1(i, pieces):
        dep = None
        off = i * RB1
        for n in _pieces(RB1, pieces):
            xn, v = layernorm(x_v[off:off + n, :].astype(F32), dep)
            h_v[off:off + n, :] = (xn * (1.0 + moda_v[0:1, D:2 * D]) + moda_v[0:1, 0:D]).astype(BF16)
            dep = mark(v)
            off += n

    def qproj(rows, j, t0=0, t1=HPC):
        q = _dot(h_v[rows, :], wq_v[j, :, t0 * DH:t1 * DH])
        for t in range(t0, t1):
            q_v[j * HPC + t, rows, :] = (q[:, (t - t0) * DH:(t - t0 + 1) * DH] * Q_SCALE).astype(BF16)

    with _scope('pro'):
        wq_copy(0).wait()
        in_order([wq_copy(j) for j in range(1, NWC)])
        qproj(slice(0, RB1), 0, 0, HPC // 2)
        x_copy(1).wait()
        ln1(1, NP0)
        qproj(slice(0, RB1), 0, HPC // 2, HPC)
        in_order([wb_copy, wr_copy, wo_copy, *kv_copies(0, 0), *kv_copies(1, 1), wg_copy, wu_copy, wd_copy])
        for i in range(1, NB1):
            if i <= 2:
                x_copy(i + 1).wait()
            elif i == 3:
                for j in range(4, NB1):
                    x_copy(j).wait()
            if i + 1 < NB1:
                ln1(i + 1, NP1)
            qproj(slice(i * RB1, (i + 1) * RB1), 0)

    def qproj_body(j, carry):
        wq_copy(j).wait()
        qproj(slice(0, S), j)
        return carry

    with _scope('qproj'):
        lax.fori_loop(1, NWC, qproj_body, 0)

    def mod_cols(g):
        cols = pl.ds(pl.multiple_of(2 * D + g * MC, DH), MC)
        n = D // (U * S // BQ)
        state = {'row': 0, 'acc': None}

        def step(q):
            r0 = state['row']
            sc_t = jnp.concatenate([scol_v[r0:r0 + n, :]] * (MC // DH), axis=1)
            prod = wm_v[r0:r0 + n, cols].astype(F32) * sc_t
            acc = state['acc']
            for t in range(n // 8):
                acc = prod[t * 8:(t + 1) * 8] if acc is None else acc + prod[t * 8:(t + 1) * 8]
            state['row'], state['acc'] = r0 + n, acc
            dep = lax.bitcast_convert_type(acc[:, 0:DH], I32) & zero_v[...]
            q0 = pltpu.bitcast(pltpu.bitcast(q[0:16], I32) | dep, BF16)
            return jnp.concatenate([q0, q[16:]], axis=0)

        def done():
            modb_v[g] = jnp.broadcast_to(jnp.sum(state['acc'], axis=0, keepdims=True), (8, MC))

        return step, done

    def fast_body(g, bad):
        slot = g & 1
        step, done = mod_cols(g)
        for u in range(U):
            bad = bad + _attn_head_fast(q_v.at[g * U + u], k_v.at[slot, u], v_v.at[slot, u],
                                        o_v.at[g * U + u], step)
        done()

        @pl.when(g + 1 < NG)
        def _():
            for cp in kv_copies(g + 1, 1 - slot):
                cp.wait()

        @pl.when(g + 2 < NG)
        def _():
            for cp in kv_copies(g + 2, slot):
                cp.start()

        return bad

    def exact_body(g, carry):
        slot = g & 1

        @pl.when(g + 1 < NG)
        def _():
            for cp in kv_copies(g + 1, 1 - slot):
                cp.start()

        for cp in kv_copies(g, slot):
            cp.wait()

        def block(n, carry):
            u = n // (S // BQX)
            _attn_rows_exact(q_v.at[g * U + u], k_v.at[slot, u], v_v.at[slot, u], o_v.at[g * U + u],
                             n % (S // BQX))
            return carry

        return lax.fori_loop(0, U * S // BQX, block, carry)

    wb_copy.wait()
    for cp in kv_copies(0, 0):
        cp.wait()
    with _scope('attn'):
        bad = lax.fori_loop(0, NG, fast_body, jnp.zeros((8, DH), F32))
    n_bad = jnp.sum(jnp.where(bad == 0.0, 0, 1))

    @pl.when(n_bad > 0)
    def _():
        for cp in kv_copies(0, 0):
            cp.start()
        lax.fori_loop(0, NG, exact_body, 0)

    def modb(j):
        per = D // MC
        return jnp.concatenate([modb_v[j * per + t][0:1, :] for t in range(per)], axis=1)

    wr_copy.wait()
    wo_copy.wait()
    wr = jnp.concatenate([wr_v[j:j + 1, :] for j in range(D // DH)], axis=1).astype(F32)
    gate_a, shift_b, scale_b, gate_b = modb(0), modb(1), _r16(1.0 + modb(2)), modb(3)
    sub8 = lax.broadcasted_iota(I32, (8, DH), 0)

    def oproj(i, dst):
        rows = pl.ds(pl.multiple_of(i * RB3, RB3), RB3)
        o = jnp.concatenate([o_v[hd, rows, :] for hd in range(H)], axis=1)
        dst[...] = _dot(o, wo_v[...])

    def finish(i, src, top, pieces):
        t1, i1, t2, i2 = top
        live = i >= 0
        base = jnp.maximum(i, 0) * RB3
        dep = None
        off = 0
        for n in _pieces(RB3, pieces):
            rows = pl.ds(pl.multiple_of(base + off, 8), n)
            x1 = x_v[rows, :].astype(F32) + gate_a * src[off:off + n, :]
            xn, _ = layernorm(x1, dep, True)
            h2 = xn * scale_b + shift_b
            h_v[rows, :] = h2.astype(BF16)
            r = _r16(jnp.sum(h2 * wr, axis=1, keepdims=True))
            y_v[rows, :] = (x1 + gate_b * (h2 + h2 * 0.0)).astype(BF16)
            dep = mark(r)
            r = jnp.where(live, r, -jnp.inf)
            for t in range(n // 8):
                rt = jnp.broadcast_to(r[t * 8:(t + 1) * 8], (8, DH))
                idx = sub8 + (base + off + t * 8)
                g1 = rt > t1
                g2 = rt > t2
                t2 = jnp.where(g1, t1, jnp.where(g2, rt, t2))
                i2 = jnp.where(g1, i1, jnp.where(g2, idx, i2))
                t1 = jnp.where(g1, rt, t1)
                i1 = jnp.where(g1, idx, i1)
            off += n
        return t1, i1, t2, i2

    def oproj_body(j, top):
        top = finish(2 * j - 1, att_b, top, NP3)
        oproj(2 * j, att_a)

        @pl.when(j > 0)
        def _():
            out_copy(2 * j - 1).start()

        top = finish(2 * j, att_a, top, NP3)
        oproj(2 * j + 1, att_b)
        out_copy(2 * j).start()
        return top

    ninf = jnp.full((8, DH), -jnp.inf, F32)
    none = jnp.full((8, DH), S, I32)
    with _scope('oproj'):
        top = lax.fori_loop(0, NB3 // 2, oproj_body, (ninf, none, ninf, none))
    for i in range(NB3 - 1):
        out_copy(i).wait()
    wg_copy.wait()
    wu_copy.wait()
    wd_copy.wait()
    with _scope('fin'):
        t1, i1, t2, i2 = finish(NB3 - 1, att_b, top, 1)
    out_copy(NB3 - 1).start()

    m1 = jnp.max(t1, axis=0, keepdims=True)
    a1 = jnp.min(jnp.where(t1 == m1, i1, S), axis=0, keepdims=True)
    won = i1 == a1
    t1b = jnp.where(won, t2, t1)
    i1b = jnp.where(won, i2, i1)
    m2 = jnp.max(t1b, axis=0, keepdims=True)
    a2 = jnp.min(jnp.where(t1b == m2, i1b, S), axis=0, keepdims=True)
    idx1 = jnp.minimum(a1[0, 0], S - 1)
    idx2 = jnp.minimum(a2[0, 0], S - 1)

    def slab(idx):
        return pl.ds(pl.multiple_of(idx & ~15, 16), 16)

    sub = lax.broadcasted_iota(I32, (16, D), 0)

    def pick_row(idx):
        rows = h_v[slab(idx), :].astype(F32)
        return jnp.sum(jnp.where(sub == (idx & 15), rows, 0.0), axis=0, keepdims=True)

    xs = jnp.where(sub == 0, pick_row(idx1), jnp.where(sub == 1, pick_row(idx2), 0.0)).astype(BF16)

    with _scope('ffn'):
        g = _dot(xs, wg_v[...])
        u = _dot(xs, wu_v[...])
        a = (g * jax.nn.sigmoid(g) * u).astype(BF16)
        y = _dot(a, wd_v[:, 0:D])
    d1 = gate_b * (y[0:1] * jax.nn.sigmoid(m1[:, 0:1]))
    d2 = gate_b * (y[1:2] * jax.nn.sigmoid(m2[:, 0:1]))

    out_copy(NB3 - 1).wait()
    for idx, d in ((idx1, d1), (idx2, d2)):
        rows = slab(idx)
        y_v[rows, :] = (y_v[rows, :].astype(F32) + jnp.where(sub == (idx & 15), d, 0.0)).astype(BF16)
    patch = [pltpu.make_async_copy(y_v.at[slab(idx), :], out_hbm.at[0, slab(idx), :], misc_sem.at[3 + n])
             for n, idx in enumerate((idx1, idx2))]
    patch[0].start()

    @pl.when((idx1 >> 4) != (idx2 >> 4))
    def _():
        patch[1].start()
        patch[1].wait()

    patch[0].wait()


@jax.jit
def pallas_adaLN_cond__mha_block_cached__moe_arch_mod__prompt_kernel(
    A_x: jax.Array,
    A_k_cache: jax.Array,
    A_v_cache: jax.Array,
    A_wq: jax.Array,
    A_wo: jax.Array,
    B_x: jax.Array,
    B_w_r: jax.Array,
    B_w_gate: jax.Array,
    B_w_up: jax.Array,
    B_w_down: jax.Array,
    c: jax.Array,
    w_mod: jax.Array,
):
    del B_x
    any_spec = pl.BlockSpec(memory_space=pl.ANY)
    scratch = [
        pltpu.VMEM((S, D), BF16),
        pltpu.VMEM((S, D), BF16),
        pltpu.VMEM((H, S, DH), BF16),
        pltpu.VMEM((H, S, DH), BF16),
        pltpu.VMEM((2, U, S, DH), BF16),
        pltpu.VMEM((2, U, S, DH), BF16),
        pltpu.VMEM((NWC, D, WC), BF16),
        pltpu.VMEM((H * DH, D), BF16),
        pltpu.VMEM((D, 6 * D + PAD), BF16),
        pltpu.VMEM((D, F), BF16),
        pltpu.VMEM((D, F), BF16),
        pltpu.VMEM((F, D + PAD), BF16),
        pltpu.VMEM((1, D), BF16),
        pltpu.VMEM((D // DH, DH), BF16),
        pltpu.VMEM((8, 2 * D), F32),
        pltpu.VMEM((NG, 8, MC), F32),
        pltpu.VMEM((D, DH), F32),
        pltpu.VMEM((RB3, D), F32),
        pltpu.VMEM((RB3, D), F32),
        pltpu.VMEM((S, D), BF16),
        pltpu.VMEM((8, DH), I32),
        pltpu.SemaphoreType.DMA((2, 2)),
        pltpu.SemaphoreType.DMA((NB1,)),
        pltpu.SemaphoreType.DMA((NKC,)),
        pltpu.SemaphoreType.DMA((NWC,)),
        pltpu.SemaphoreType.DMA((4,)),
        pltpu.SemaphoreType.DMA((5,)),
        pltpu.SemaphoreType.DMA((NB3,)),
        pltpu.SemaphoreType.REGULAR,
    ]
    return pl.pallas_call(
        _kernel,
        out_shape=jax.ShapeDtypeStruct((1, S, D), BF16),
        in_specs=[any_spec] * 11,
        out_specs=any_spec,
        scratch_shapes=scratch,
        compiler_params=pltpu.CompilerParams(vmem_limit_bytes=122 * 1024 * 1024),
    )(A_x, A_k_cache, A_v_cache, A_wq, A_wo, B_w_r.reshape(D // DH, DH), B_w_gate, B_w_up, B_w_down,
      c, w_mod)
```
